```python
import os as _os
_os.environ.setdefault("JAX_PLATFORMS", "cpu")
import jax
import jax.numpy as jnp

def _softmax(x, axis=-1):
    return jax.nn.softmax(x, axis=axis)
def _gelu(x):
    return jax.nn.gelu(x, approximate=True)
def _silu(x):
    return jax.nn.silu(x)
def _sigmoid(x):
    return jax.nn.sigmoid(x)
def _layernorm(x, axis=-1, eps=1e-5):
    m = jnp.mean(x, axis=axis, keepdims=True)
    v = jnp.var(x, axis=axis, keepdims=True)
    return (x - m) / jnp.sqrt(v + eps)
def _scatter_add(tgt, idx, src, axis=0):
    return tgt.at[idx].add(src)
def _segment_sum(src, seg, n):
    return jax.ops.segment_sum(src, seg, n)
class _Rng:
    def __init__(self, key):
        self._k = key
    def _next(self):
        self._k, sub = jax.random.split(self._k)
        return sub
    def normal(self, shape):
        return jax.random.normal(self._next(), shape, dtype=jnp.bfloat16)
    def randint(self, lo, hi, shape):
        return jax.random.randint(self._next(), shape, lo, hi, dtype=jnp.int32)
    def uniform(self, shape, lo=0.0, hi=1.0):
        return jax.random.uniform(self._next(), shape, jnp.bfloat16, lo, hi)
    def permutation(self, n):
        return jax.random.permutation(self._next(), n)


kernel_name = 'concat_heads__grouped_kv_mqa__sliding_block__prompt'

def setup_inputs():
    _rng = _Rng(jax.random.key(int.from_bytes(__import__("os").urandom(4), "little")))
    _w = (lambda a: (lambda t: t.astype(jnp.bfloat16) if jnp.issubdtype(t.dtype, jnp.floating) else t)(jnp.asarray(a)))
    def _A_setup():
        B, S, D, H = 1, 2048, 576, 32
        Dh = D // H
        return {
            "x": _w((lambda *s: _rng.normal(s) * 0.05)(B, S, D)),
            "wq": _w((lambda *s: _rng.normal(s) * 1.6)(D, H * Dh)),
            "wk": _w((lambda *s: _rng.normal(s) * 1.6)(D, Dh)),
            "wv": _w((lambda *s: _rng.normal(s) * 0.1)(D, Dh)),
            "wo": _w((lambda *s: _rng.normal(s) * 0.1)(H * Dh, D)),
        }
    _A_in = _A_setup()

    def _B_setup():
        B, S, D = 1, 2048, 576
        return {
            "x": _w((lambda *s: _rng.normal(s) * 0.2)(B, S, D)),
            "wqkv": _w((lambda *s: _rng.normal(s) * 0.2)(D, 3 * D)),
            "wo": _w((lambda *s: _rng.normal(s) * 0.05)(D, D)),
        }
    _B_in = _B_setup()

    return {
        "A_x": _A_in["x"],
        "A_wq": _A_in["wq"],
        "A_wk": _A_in["wk"],
        "A_wv": _A_in["wv"],
        "A_wo": _A_in["wo"],
        "B_x": _B_in["x"],
        "B_wqkv": _B_in["wqkv"],
        "B_wo": _B_in["wo"],
    }

def reference(A_x, A_wq, A_wk, A_wv, A_wo, B_x, B_wqkv, B_wo):
    def _A_ref(x, wq, wk, wv, wo):
        B, S, D = x.shape
        H = 32
        Dh = D // H
        q = (lambda x, *d: x.transpose(*d))((x @ wq).reshape(B, S, H, Dh), 0, 2, 1, 3)
        k = x @ wk
        v = x @ wv
        scores = jnp.einsum("bhqd,bkd->bhqk", q, k) * (Dh ** -0.5)
        p = _softmax(scores, axis=-1)
        o = jnp.einsum("bhqk,bkd->bhqd", p, v)
        return (lambda x, *d: x.transpose(*d))(o, 0, 2, 1, 3).reshape(B, S, H * Dh) @ wo

    def _B_ref(x, wqkv, wo):
        B, S, D = x.shape
        H = 32; Dh = D // H; W = 256
        qkv = (lambda x, *d: x.transpose(*d))((x @ wqkv).reshape(B, S, 3, H, Dh), 2, 0, 3, 1, 4)
        q, k, v = qkv[0], qkv[1], qkv[2]
        scores = jnp.einsum("bhqd,bhkd->bhqk", q, k) * (Dh ** -0.5)
        idx = jnp.arange(S)
        mask = (idx[:, None] - idx[None, :] >= 0) & (idx[:, None] - idx[None, :] < W)
        scores = jnp.where(mask[None, None], scores, -1e9)
        p = _softmax(scores, axis=-1)
        o = jnp.einsum("bhqk,bhkd->bhqd", p, v)
        return (lambda x, *d: x.transpose(*d))(o, 0, 2, 1, 3).reshape(B, S, D) @ wo

    a = _A_ref(A_x, A_wq, A_wk, A_wv, A_wo)
    b = _B_ref(B_x, B_wqkv, B_wo)
    return jnp.concatenate([a, b], axis=-1)
```

```python
import functools

import jax
import jax.numpy as jnp
import numpy as np
from jax import lax
from jax.experimental import pallas as pl
from jax.experimental.pallas import tpu as pltpu

S, D, H, DH = 2048, 576, 32, 18
T = 128
NT = 4
QB = NT * T
NSB = S // QB
NC = S // T
DK = 640
U = 8
NG = H // U
GR = U * DH
UN = 2
RO = 48
WCUT = (0, 640, 1280, 3 * D)
F32, BF16, I32 = jnp.float32, jnp.bfloat16, jnp.int32
QSCALE = float(DH ** -0.5 * np.log2(np.e))
NEG = -1e30
L_LO, L_HI = 2.0 ** -24, 2.0 ** 100

NM = NC - 3
VKEYS = [16 * (c == 7) for c in range(NM)] + [T] * (NC - NM)
VOFF = [sum(VKEYS[:c]) for c in range(NC + 1)]
TILE = [sorted(range(NC), key=lambda c: -VKEYS[c]).index(c) for c in range(NC)]
KA0, VA0 = 0, S // 2
KB0 = VA0 + NC * 24


def _matmul_order():
    events, due_v, due_w, slot, taken = [], [(-1, NM - 1)], [(-1, NC - 1)], 0, 0
    for u in range(U):
        order = ""
        for ch in "PqvbvBcqCqvPqvqvqvPqvqvqvqv" if u else "qwvqvqvpppppvqwqvqvqvqwvqvqvbvBcqCqvqv":
            if ch == "P":
                slot += 1
                n = (slot * 6 + 10) // 21 - taken
                taken += n
                ch = "ovqw" if n else "qwv"
            order += ch
        c, first_w = 0, True
        for ch in order:
            if ch == "q":
                events.append(("q", u, c, T - VKEYS[c]))
                due_v.append((u, c))
                c += 1
            elif ch == "v":
                events.append(("v", *due_v.pop(0), 24))
            elif ch == "w":
                events.append(("v", *due_w.pop(0), 24))
                if first_w:
                    due_w, first_w = [(u, i) for i in range(NM, NC)], False
            else:
                events.append((ch, u, 0, {"b": T, "c": 24, "B": T + 32, "C": 48, "p": 3 * GR, "o": 5 * RO}[ch]))
    return events


def _vector_work():
    items = []
    for u in range(U):
        keys = [(c, r) for c in sorted(range(NC), key=lambda c: c if c < NM else (c - NM + 0.9) * NM / (NC - NM))
                for r in range(0, VKEYS[c], 16)]
        n = -(-len(keys) // 3)
        for b in range(n):
            rows = [(c, r + a) for c, r in keys[b * len(keys) // n:(b + 1) * len(keys) // n] for a in (0, 8)]
            items += [(u, c, r, j, part) for j in (0, 2) for part in range(3) for c, r in rows]
    return items


PACING = (
    [12, 1, 2, 17, 1, 13, 1, 54, 54, 53, 56, 55, 3, 8, 6, 14, 3, 15, 4, 15, 2, 10, 7, 3, 13, 5, 8, 3, 15, 4, 13, 5, 5,
     6, 15, 3, 14, 4, 13, 3, 2, 15, 1, 14, 4, 16, 3, 10, 6, 13, 1, 3, 5, 5, 5, 6, 2, 11, 2, 15, 3, 15, 2, 12, 3, 11,
     3, 2, 15, 3, 14, 2, 15, 3, 15, 2, 12, 3, 3, 14, 2, 13, 4, 12, 3, 16, 3, 15, 1, 11, 2, 3, 15, 2, 15, 1, 15, 2,
     7, 5, 5, 5, 5, 1, 11, 2, 16, 2, 15, 1, 15, 3, 14, 3, 14, 6, 1, 17, 1, 8, 5, 17, 1, 9, 5, 15, 1, 11, 4, 3, 15,
     2, 14, 2, 13, 3, 3, 5, 3, 5, 5, 6, 12, 7, 13, 2, 8, 5, 14, 4, 15, 2, 11, 3, 4, 14, 3, 13, 6, 12, 3, 9, 5, 15,
     2, 11, 1, 4, 17, 2, 16, 1, 12, 2, 11, 4, 2, 15, 3, 14, 3, 14, 3, 14, 4, 5, 4, 3, 5, 5, 2, 14, 2, 16, 1, 13, 4,
     14, 3, 11, 3, 14, 1, 15, 3, 3, 14, 3, 14, 3, 13, 3, 12, 1, 3, 14, 3, 15, 1, 16, 2, 15, 5, 5, 5, 3, 4, 5, 3, 11,
     3, 15, 0, 13, 2, 17, 3, 11, 5, 15, 1, 11, 4, 3, 15, 2, 15, 2, 13, 3, 11, 9, 2, 13, 0, 11, 2, 16, 3, 14, 3, 12,
     5, 3, 14, 1, 14, 3, 21, 3, 5, 3, 15, 0, 3, 6, 5, 6, 5, 3, 13, 3, 14, 3, 13, 3, 10, 3, 9, 2, 2, 12, 3, 12, 2,
     12, 3, 0, 0],
    [14, 2, 2, 15, 0, 12, 2, 54, 70, 56, 42, 49, 0, 16, 2, 15, 3, 15, 2, 15, 2, 11, 3, 3, 13, 3, 8, 6, 15, 5, 14, 3, 10,
     3, 16, 3, 14, 3, 14, 2, 4, 13, 2, 14, 3, 16, 3, 10, 5, 13, 3, 3, 6, 3, 6, 6, 1, 12, 2, 15, 3, 15, 2, 12, 3, 11,
     3, 2, 15, 3, 14, 2, 15, 3, 15, 2, 12, 3, 3, 14, 2, 13, 4, 18, 0, 10, 4, 15, 1, 11, 4, 3, 15, 2, 15, 1, 15, 3,
     6, 5, 5, 5, 5, 1, 11, 2, 16, 2, 15, 1, 16, 3, 14, 2, 14, 6, 2, 13, 1, 9, 4, 16, 3, 10, 3, 17, 1, 12, 4, 3, 15,
     3, 14, 2, 13, 2, 3, 5, 6, 5, 6, 3, 14, 1, 15, 3, 12, 3, 14, 3, 15, 1, 11, 3, 4, 14, 3, 13, 6, 15, 3, 9, 5, 13,
     3, 11, 2, 2, 17, 2, 15, 1, 12, 3, 11, 3, 2, 15, 3, 14, 3, 14, 3, 16, 4, 3, 4, 5, 6, 4, 1, 13, 2, 16, 1, 13, 4,
     15, 3, 10, 3, 14, 1, 15, 3, 3, 14, 5, 14, 3, 13, 2, 10, 2, 3, 15, 3, 15, 0, 16, 3, 15, 4, 4, 5, 3, 5, 5, 3, 11,
     3, 14, 1, 13, 2, 17, 3, 11, 5, 15, 0, 12, 4, 3, 15, 2, 15, 2, 13, 3, 11, 3, 2, 16, 3, 11, 3, 13, 3, 14, 3, 15,
     4, 3, 16, 1, 8, 2, 21, 2, 10, 4, 15, 0, 3, 6, 5, 8, 5, 1, 13, 3, 14, 3, 13, 3, 10, 3, 9, 2, 2, 12, 3, 12, 1,
     13, 3, 0, 0],
)


def _dot(a, b):
    return lax.dot_general(a, b, (((1,), (0,)), ((), ())), preferred_element_type=F32)


def _i32(x):
    return pltpu.bitcast(x, I32)


def _f32(x):
    return pltpu.bitcast(x, F32)


def _bf16(x):
    return pltpu.bitcast(x, BF16)


def _project(w, x):
    y = None
    for k in range(0, DK, T):
        d = _dot(_bf16(w[:, k:k + T]), x(k, k + T))
        y = d if y is None else y + d
    return y


def _transpose_into(dst, r0, src, c0, n):
    for c in range(0, n, T):
        cw = min(T, n - c)
        x = jnp.concatenate([src[:, c0 + c:c0 + c + cw], jnp.zeros((DK - D, cw), BF16)], axis=0)
        dst[(r0 + c) // 2:(r0 + c + cw) // 2, :] = _i32(x.T)


def _flip(x, n):
    return jnp.concatenate([x[r:r + n] for r in range(x.shape[0] - n, -1, -n)], axis=0)


def _pack32(x):
    return jnp.concatenate([x, jnp.zeros((8, x.shape[1]), F32)], axis=0).astype(BF16)


def _kernel(pacing, xa_h, wq_h, wk_h, wv_h, woa_h, xb_h, wqkv_h, wob_h, out_h,
            xa, xb, wq, wk, wv, woa, wob, wqkv,
            xp, wbt, wot, qa, kt, akv, qkv, vh, kh, ot, ostage, pc, ac, chk, zero, sems, osems):
    def xcopy(src, dst, i, base):
        return pltpu.make_async_copy(src.at[:, pl.ds(i * QB, QB)], dst.at[:, pl.ds(i * QB, QB)], sems.at[base + i])

    cp_w = [pltpu.make_async_copy(s, d, sems.at[8 + i]) for i, (s, d) in enumerate(
        [(wq_h, wq), (wk_h, wk), (wv_h, wv)]
        + [(wqkv_h.at[:, c0:c1], wqkv.at[:, c0:c1]) for c0, c1 in zip(WCUT, WCUT[1:])]
        + [(woa_h, woa), (wob_h, wob)])]
    for cp in (cp_w[0], cp_w[1], cp_w[2], xcopy(xa_h, xa, 0, 0), xcopy(xa_h, xa, 1, 0), cp_w[3],
               xcopy(xa_h, xa, 2, 0), cp_w[4], xcopy(xa_h, xa, 3, 0), cp_w[5], xcopy(xb_h, xb, 0, 4),
               cp_w[6], cp_w[7], xcopy(xb_h, xb, 1, 4), xcopy(xb_h, xb, 2, 4), xcopy(xb_h, xb, 3, 4)):
        cp.start()

    def clear(i, _):
        zero[i] = 0
        return 0
    lax.fori_loop(0, 2, clear, 0)

    row8 = lax.broadcasted_iota(I32, (8, T), 0)
    lane8 = lax.broadcasted_iota(I32, (8, T), 1)
    zeros8 = jnp.zeros((8, T), F32)

    kh[2 * H * 2] = _i32(jnp.where(lax.broadcasted_iota(I32, (T, T), 1) % 32 == DH, 1.0, 0.0).astype(BF16))
    vh[2 * NG * 2] = jnp.zeros((GR + 8, T), F32)
    chk[...] = jnp.ones(chk.shape, F32)
    ac[...] = jnp.ones(ac.shape, F32)
    pc[...] = jnp.zeros(pc.shape, I32)

    def head_rows(ref, b, r, fill):
        last = jnp.concatenate([ref[b, pl.ds(r + 16, 2), :], fill[2:8]], axis=0)
        return jnp.concatenate([ref[b, pl.ds(r, 16), :], last], axis=0)

    def values_a(c):
        return _f32(akv[VA0 + 24 * TILE[c]:VA0 + 24 * TILE[c] + 24, :])

    def weights_b(g, part, k0, k1):
        return wbt[pl.ds(pl.multiple_of(part * D // 2 + g * (GR // 2), 8), GR // 2), k0:k1]

    def normalize(acc, js, par, p, g, u, seen):
        for n, j in enumerate(js):
            a = acc[:, n * T:(n + 1) * T]
            l = a[16:24]
            seen[:] = jnp.minimum(seen[0], l), jnp.maximum(seen[1], l), seen[2] + (a[0:8] + a[8:16] + l)
            r = pltpu.reciprocal(l, approx=True)
            r = r * (2.0 - l * r)
            ot[par, p, j, g, u * DH:(u + 1) * DH, :] = (a * r[2:3])[0:DH]

    def project_out(slot, heads, n, rows, pace, keep=None):
        for i in range(4):
            r0 = (4 * n + i) * RO
            y = _dot(_bf16(pace(wot[r0 // 2:(r0 + RO) // 2, :], 4)), heads[r0 // D])
            if keep is not None:
                qa[keep + r0 // GR, r0 % GR:r0 % GR + RO, :] = y
            rows += [y[r:r + 16] for r in range(0, RO, 16)]
        c0 = (4 * n + 4) * RO - 16 * len(rows)
        t0 = slot * T if isinstance(slot, int) else pl.multiple_of(slot * T, T)
        while len(rows) >= T // 16:
            ostage[pl.ds(t0, T), c0:c0 + T] = jnp.concatenate(rows[:T // 16], axis=0).astype(BF16).T
            del rows[:T // 16]
            c0 += T

    def output_tile(slot, par, j):
        pad = [jnp.zeros((DK - D, T), F32)]
        heads = [jnp.concatenate([ot[par, p, j, g, 0:GR, :] for g in range(NG)] + pad, axis=0).astype(BF16)
                 for p in range(2)]
        rows = []
        for n in range(2 * D // (4 * RO)):
            project_out(slot, heads, n, rows, lambda x, cycles: x)

    def out_copy(t, slot, n):
        return pltpu.make_async_copy(ostage.at[pl.ds(slot * T, n * T)], out_h.at[pl.ds(t * T, n * T)], osems.at[slot])

    def attend_groups(sb, g0, pk, qbc, kr):
        carry = [[pc[n * NT + j] for j in range(NT)] for n in range(2)] + [ac[...], [chk[0], chk[1], chk[2]]]
        for i in range(UN):
            carry = attend_group(sb, g0, i, carry, pk, qbc, kr.at[i], qkv.at[i], pacing[i])
        always = jnp.concatenate([lane8 + zero[1] < T] * 8, axis=0)
        for n in range(3):
            chk[n] = carry[3][n]
        for j in range(NT):
            pc[j] = carry[0][j]
            late = jnp.concatenate([_i32(carry[2][0:8, j * T:(j + 1) * T])] * 8, axis=0)
            pc[NT + j] = jnp.where(always, carry[1][j], late)
        ac[...] = carry[2]

    def attend_group(sb, g0, i, carry, pk, qbc, kr, cur, counts):
        g = g0 + i
        it = sb * NG + g
        par = sb % 2
        blk = [(sb * NT + j) * NG + g for j in range(NT)]
        z = zero[0]
        always = lane8 + z < T
        lane16 = lax.broadcasted_iota(I32, (16, T), 1)
        ones = jnp.where(row8 == 2, 1.0, 0.0)
        seen = carry[3]
        probs = {}

        def start_sum(n):
            return jnp.full((24, n), z.astype(F32), F32)

        def pack(p):
            pk[0:p.shape[0] // 2, 0:p.shape[1]] = _i32(p.astype(BF16))
            return pk[0:p.shape[0] // 2, 0:p.shape[1]]

        def put(key, j, r, p):
            probs.setdefault((key, j), {})[r] = p

        def take(key, j):
            parts = probs.pop((key, j))
            return jnp.concatenate([parts[r] for r in sorted(parts)], axis=0)

        def spread_q(u, d0, d1):
            for d in range(d0, d1):
                for j in range(NT):
                    r0 = u % U * DH + d // 8 * 8
                    rows = qa[blk[j] + 1 if u == U else blk[j], r0:r0 + (8 if d < 16 else 2), :]
                    row = rows[d % 8:d % 8 + 1]
                    qbc[i * U + u, d * 8:d * 8 + 8, j * T:(j + 1) * T] = jnp.broadcast_to(row, (8, T))
        if i == 0:
            spread_q(0, 0, DH)
        work, partial, qs = _vector_work(), {}, {}

        def vector_item(n):
            u, c, r, j0, part = work[n]
            r0 = KB0 + ((VOFF[c] + r) // 8 * DH + part * 6) * 8
            k = _f32(akv[r0:r0 + 48, :])
            if (u, part, j0) not in qs:
                qs[u, part, j0] = qbc[i * U + u, part * 48:(part + 1) * 48, j0 * T:(j0 + 2) * T]
            k = jnp.concatenate([k, k], axis=1)
            s = partial.pop((c, r), None)
            for d in range(0, 48, 8):
                t = k[d:d + 8] * qs[u, part, j0][d:d + 8]
                s = t if s is None else s + t
            if part < 2:
                partial[c, r] = s
                done = [_i32(s)]
            elif r % 16 == 0:
                partial[c, r, "p"] = jnp.exp2(s)
                done = []
            else:
                done = [pack(jnp.concatenate([partial.pop((c, r - 8, "p")), jnp.exp2(s)], axis=0))]
                for j in range(2):
                    put((u, c), j0 + j, (T - VKEYS[c] + r - 8) // 2, done[0][:, j * T:(j + 1) * T])
            per = len(work) // U
            if i * U + u + 1 < UN * U:
                spread_q(u + 1, n % per * DH // per, (n % per + 1) * DH // per)
            return done

        clock = {"done": 0, "first": 0}

        def pace(x, cycles, also=None):
            cols = []
            for c0 in range(0, x.shape[1], T):
                rows = []
                for r0 in range(0, x.shape[0], 8):
                    y = x[r0:r0 + 8, c0:c0 + T]
                    clock["t"] += cycles
                    k, rest = divmod(clock["t"], clock["span"])
                    k += clock["first"]
                    target = sum(counts[:k]) + (counts[k] * rest // clock["span"] if rest else 0)
                    due = [p for n in range(clock["done"], target) for p in vector_item(n)]
                    clock["done"] = target
                    if due:
                        p = functools.reduce(jnp.bitwise_or, due)
                        due = [p[:, 0:T], p[:, T:2 * T]]
                    if also is not None:
                        due.append(also[r0:r0 + 8])
                    if due:
                        p = functools.reduce(jnp.bitwise_or, due)
                        y = jnp.where(always, y, p if y.dtype == I32 else _f32(p))
                    rows.append(y)
                cols.append(jnp.concatenate(rows, axis=0))
            return jnp.concatenate(cols, axis=1)

        def queries_a(u):
            q = jnp.concatenate([head_rows(qa, blk[j], u * DH, zeros8) for j in range(NT)], axis=1)
            return jnp.concatenate([q, jnp.zeros((T - 24, QB), F32)], axis=0).astype(BF16)

        st = [{} for _ in range(U)] + [{"n": NC - 2, "acc": carry[2]}]
        for n, c in enumerate((NM - 1, NC - 1)):
            for j in range(NT):
                put((-1, c), j, 0, carry[n][j])
        st[0]["q"] = queries_a(0)
        fetched, heads, out_rows = [], [], []

        def scores_a(u, c):
            if c == NM - 1 and u + 1 < U:
                st[u + 1]["q"] = queries_a(u + 1)
            rows = range(T - VKEYS[c] - 16, -1, -16)
            k = [akv[r0:r0 + 8, :] for r0 in (KA0 + (TILE[c] * T + r) // 2 for r in rows)]
            also = None
            if len(fetched) < 2 * NG and u * NM + c >= 2:
                p, g2 = divmod(len(fetched), NG)
                also = jnp.concatenate([pack(ot[1 - par, p, g, g2, r:r + RO, :]) for r in range(0, GR, RO)], axis=0)
                fetched.append(also)
            p = jnp.exp2(_dot(_bf16(pace(jnp.concatenate(k, axis=0), 16, also)), st[u]["q"]))
            for n, r in enumerate(rows):
                x = p[16 * n:16 * n + 16]
                if VKEYS[c] or (i, u, c) == (UN - 1, U - 1, NM - 1):
                    x = pack(x)
                for j in range(NT):
                    put((u, c), j, r // 2, x[:, j * T:(j + 1) * T])

        def sum_a(u, c):
            v = pace(values_a(c), 8)
            p = jnp.concatenate([take((u, c), j) for j in range(NT)], axis=1)
            d = _dot(v, p if p.dtype == F32 else _bf16(p))
            st[u]["n"] = st[u].get("n", 0) + 1
            st[u]["acc"] = st[u].get("acc", start_sum(QB)) + d
            if st[u]["n"] == NC and u < 0:
                normalize(st[u]["acc"], range(NT), (it - 1) // NG % 2, 0, jnp.where(it == 0, NG, (it - 1) % NG),
                          U - 1, seen)
            elif st[u]["n"] == NC:
                normalize(st[u]["acc"], range(NT), par, 0, g, u, seen)

        def project_b(*_):
            k = clock["k"] = clock.get("k", -T) + T
            w = jnp.concatenate([weights_b(g, part, k, k + T) for part in range(3)], axis=0)
            y = _dot(_bf16(pace(w, 16)), _bf16(xp[k // 2:(k + T) // 2, :]))
            y = clock["y"] = clock["y"] + y if k else y
            if k + T < DK:
                return
            for part in range(3):
                x = y[part * GR:(part + 1) * GR] * QSCALE if part == 0 else y[part * GR:(part + 1) * GR]
                for j in range(NT):
                    cur[part * NT + j, 0:GR, :] = x[:, j * T:(j + 1) * T]
                    if part == 2 and j >= NT - 2:
                        vh[(par * NG + g) * 2 + j - (NT - 2), 0:GR, :] = x[:, j * T:(j + 1) * T]
                if part == 1:
                    for u in range(U):
                        for j in range(NT):
                            k = pack(jnp.concatenate([head_rows(cur, NT + j, u * DH, zeros8), zeros8], axis=0))
                            k = _i32(_bf16(jnp.concatenate([k] * 4, axis=0)).T)
                            kr[u * NT + j] = k
                            if j >= NT - 2:
                                kh[(par * H + g * U + u) * 2 + j - (NT - 2)] = k

        def keys_b(u, j):
            if j >= 2:
                return kr[u * NT + j - 2]
            return kh[jnp.where(sb == 0, 2 * H * 2, ((1 - par) * H + g * U + u) * 2 + j)]

        def values_b(u, j):
            if j >= 2:
                return head_rows(cur, 2 * NT + j - 2, u * DH, ones)
            return head_rows(vh, jnp.where(sb == 0, 2 * NG * 2, ((1 - par) * NG + g) * 2 + j), u * DH, ones)

        def queries_b(u, j):
            if ("q", j) not in st[u]:
                q = head_rows(cur, j, u * DH, jnp.where(row8 == 2, NEG, 0.0))
                q = pack(jnp.concatenate([q, zeros8], axis=0))
                st[u]["q", j] = _bf16(jnp.concatenate([jnp.where(lane16 // 32 == n, q, 0) for n in range(4)], axis=0))
            return st[u]["q", j]

        def scores_mid(u, _):
            for j in range(NT):
                k = _flip(keys_b(u, j + 1), 8)
                if j == 0:
                    k = pace(k, 16)
                put("mid", j, 0, jnp.exp2(_flip(_dot(_bf16(k), queries_b(u, j)), 16)))

        def sum_mid(u, _):
            for j in range(NT):
                v = pace(values_b(u, j + 1), 2)
                st[u]["b", j] = start_sum(T) + _dot(v, take("mid", j))

        def scores_edge(u, _):
            row = lax.broadcasted_iota(I32, (32, T), 0)
            lane = lax.broadcasted_iota(I32, (32, T), 1)
            row2 = 2 * lax.broadcasted_iota(I32, (T // 2, T), 0)
            lane2 = lax.broadcasted_iota(I32, (T // 2, T), 1)
            newest = jnp.where(row2 <= lane2, 0xFFFF, 0) | jnp.where(row2 + 1 <= lane2, -0x10000, 0)
            for j in range(NT):
                old, new = keys_b(u, j), keys_b(u, j + 2)
                mixed = [new[0:16]] + [
                    jnp.where(lane16 >= 32 * n, new[16 * n:16 * n + 16], old[16 * n:16 * n + 16]) for n in range(1, 4)]
                diag = old[0:16]
                for n in range(1, 4):
                    diag = jnp.where(lane16 >= 32 * n, old[16 * n:16 * n + 16], diag)
                k = jnp.concatenate([diag, _flip(jnp.concatenate(mixed, axis=0), 8)], axis=0)
                if j == 0:
                    k = pace(k, 16)
                s = _dot(_bf16(k), queries_b(u, j))
                s_diag, s = s[0:32], _flip(s[32:], 16)
                s = jnp.concatenate([jnp.where((lane >= 32 * n) & (lane < row + 32 * n), s_diag, s[32 * n:32 * n + 32])
                                     for n in range(4)], axis=0)
                p = pack(jnp.exp2(s))
                p_new = p & newest
                put(0, j, 0, p ^ p_new)
                put(1, j, 0, p_new)

        def sum_edge(u, _):
            for n in range(2):
                for j in range(NT):
                    v = pace(values_b(u, j + 2 * n), 2)
                    st[u]["b", j] = st[u]["b", j] + _dot(v, _bf16(take(n, j)))
            for j in range(NT):
                normalize(st[u]["b", j], [j], par, 1, g, u, seen)

        def output_slice(*_):
            if not heads:
                pad = [jnp.zeros(((DK - D) // 2, T), I32)]
                heads.extend(_bf16(jnp.concatenate(fetched[p * NG:(p + 1) * NG] + pad, axis=0)) for p in range(2))
            clock["out"] = clock.get("out", -1) + 1
            project_out(g, heads, clock["out"], out_rows, pace, jnp.where(sb == 0, 2 * NT + 2 * g, NC) * NG)

        run = {"q": scores_a, "v": sum_a, "b": scores_mid, "c": sum_mid, "B": scores_edge, "C": sum_edge,
               "p": project_b, "o": output_slice}
        for kind, u, c, cycles in _matmul_order():
            stretches = 5 if kind == "o" else 1
            clock.update(t=0, span=cycles // stretches)
            run[kind](u, c)
            clock["first"] += stretches
        assert clock["done"] == len(work)
        return [[take((U - 1, c), j) for j in range(NT)] for c in (NM - 1, NC - 1)] + [st[U - 1]["acc"], seen]

    def attend_safely(t):
        row = lax.broadcasted_iota(I32, (T, T), 0)
        lane = lax.broadcasted_iota(I32, (T, T), 1)
        cur = qkv.at[0]

        def group(g, _):
            def project(i, _):
                c0 = pl.multiple_of(jnp.maximum(t + i - 2, 0) * T, T)
                x = jnp.concatenate([xb[:, pl.ds(c0, T)], jnp.zeros((DK - D, T), BF16)], axis=0)
                for part in range(3):
                    y = _project(weights_b(g, part, 0, DK), lambda k0, k1: x[k0:k1])
                    cur[part * NT + i, 0:GR, :] = y * QSCALE if part == 0 else y
                return 0
            lax.fori_loop(0, 3, project, 0)

            def head(u, _):
                r = u * DH
                q = _pack32(head_rows(qa, t * NG + g, r, zeros8))

                def chunk(c, carry):
                    m, acc = carry
                    k = _bf16(akv[pl.ds(pl.multiple_of(KA0 + c * (T // 2), 8), T // 2), :])[:, 0:32]
                    v = _f32(akv[pl.ds(pl.multiple_of(VA0 + c * 24, 8), 24), :])
                    s = _dot(k, q)
                    m_new = jnp.maximum(m, jnp.max(s, axis=0, keepdims=True))
                    return m_new, acc * jnp.exp2(m - m_new) + _dot(v, jnp.exp2(s - m_new).astype(BF16))
                _, acc = lax.fori_loop(0, NC, chunk, (jnp.full((1, T), float(np.finfo(np.float32).min), F32), jnp.zeros((24, T), F32)))
                ot[0, 0, 0, g, pl.ds(r, 24), :] = acc / acc[DH:DH + 1, :]

                q = _pack32(head_rows(cur, 2, r, zeros8))
                ss = []
                for i, inside in enumerate((row > lane, row >= 0, row <= lane)):
                    k = jnp.concatenate([head_rows(cur, NT + i, r, zeros8), jnp.zeros((T - 24, T), F32)], axis=0)
                    s = _dot(k.T.astype(BF16)[:, 0:32], q)
                    ss.append(jnp.where(inside & (t + i >= 2), s, -jnp.inf))
                m = jnp.max(jnp.maximum(jnp.maximum(ss[0], ss[1]), ss[2]), axis=0, keepdims=True)
                acc = sum(_dot(head_rows(cur, 2 * NT + i, r, jnp.where(row8 == 2, 1.0, 0.0)),
                               jnp.exp2(ss[i] - m).astype(BF16)) for i in range(3))
                ot[0, 1, 0, g, pl.ds(r, 24), :] = acc / acc[DH:DH + 1, :]
                return 0
            lax.fori_loop(0, U, head, 0)
            return 0
        lax.fori_loop(0, NG, group, 0)

    def project_kv(i, wkv):
        kv = _dot(wkv, xa[:, i * QB:(i + 1) * QB])
        k = (kv[0:24] * QSCALE).astype(BF16).astype(F32)
        kt[i * QB:(i + 1) * QB, :] = jnp.concatenate([k, jnp.zeros((T - 24, QB), F32)], axis=0).T
        akv[KA0 + i * QB // 2:KA0 + (i + 1) * QB // 2, :] = _i32(kt[i * QB:(i + 1) * QB, :].astype(BF16))
        row = lax.broadcasted_iota(I32, (24, QB), 0)
        v = _i32(jnp.where(row == DH, 1.0, kv[24:48].astype(BF16).astype(F32)))
        for j in range(NT):
            r0 = VA0 + (i * NT + j) * 24
            akv[r0:r0 + 24, :] = v[:, j * T:(j + 1) * T]

    def project_q(i, g0, g1):
        x = jnp.concatenate([xa[:, i * QB:(i + 1) * QB], jnp.zeros((DK - D, QB), BF16)], axis=0)
        for g in range(g0, g1):
            y = _project(wot[g * GR // 2:(g + 1) * GR // 2, :], lambda k0, k1: x[k0:k1])
            for j in range(NT):
                qa[(i * NT + j) * NG + g, 0:GR, :] = y[:, j * T:(j + 1) * T]

    def load_xb(c0):
        xp[0:D // 2, :] = _i32(xb[:, pl.ds(c0, QB)])

    cp_w[0].wait()
    _transpose_into(wot, 0, wq, 0, D)
    wot[D // 2:D, :] = wot[0:D // 2, :]
    cp_w[1].wait()
    cp_w[2].wait()
    pad = jnp.zeros((24 - DH, D), F32)
    wkv = jnp.concatenate([wk[...].astype(F32), pad, wv[...].astype(F32), pad], axis=0).astype(BF16)
    xcopy(xa_h, xa, 0, 0).wait()
    project_kv(0, wkv)
    project_q(0, 0, NG)
    for c in range(NC):
        for r in range(0, VKEYS[c], 16):
            r0 = (TILE[c] + 1) * T - VKEYS[c] + r
            k = kt[r0:r0 + 16, :]
            for d in range(DH):
                kd = _i32(jnp.broadcast_to(k[:, d:d + 1], (16, T)))
                for a in range(2):
                    r0 = KB0 + (((VOFF[c] + r) // 8 + a) * DH + d) * 8
                    akv[r0:r0 + 8, :] = kd[8 * a:8 * a + 8]
    xp[D // 2:DK // 2, :] = jnp.zeros(((DK - D) // 2, QB), I32)
    for i in range(1, NSB):
        xcopy(xa_h, xa, i, 0).wait()
        cp_w[2 + i].wait()
        _transpose_into(wbt, WCUT[i - 1], wqkv, WCUT[i - 1], WCUT[i] - WCUT[i - 1])
        project_kv(i, wkv)
        if i >= 2:
            x = xa[:, i * QB:(i + 1) * QB].astype(F32)
            for g in range(NG):
                for j in range(NT):
                    n = (i - 2) * NT + j
                    ot[1, n % 2, n // 2, g, 0:GR, :] = x[g * GR:(g + 1) * GR, j * T:(j + 1) * T]
        project_q(1, *((0, 2), (2, 3), (3, 4))[i - 1])
    xcopy(xb_h, xb, 0, 4).wait()
    load_xb(0)

    def step(n, _):
        it = n * UN
        sb, g = it // NG, it % NG

        @pl.when(it == NG)
        def _():
            cp_w[6].wait()
            cp_w[7].wait()
            _transpose_into(wot, 0, woa, 0, D)
            _transpose_into(wot, D, wob, 0, D)

        @pl.when(sb >= 2)
        def _():
            out_copy(it - 2 * NG, g, UN).wait()

        pl.run_scoped(functools.partial(attend_groups, sb, g),
                      pltpu.VMEM((T // 2, QB), I32), pltpu.VMEM((UN * U, DH * 8, QB), F32),
                      pltpu.VMEM((UN, U * NT, T // 2, T), I32))

        @pl.when(sb > 0)
        def _():
            out_copy(it - NG, g, UN).start()

        def next_block(*_):
            xcopy(xb_h, xb, sb + 1, 4).wait()
            load_xb(pl.multiple_of((sb + 1) * QB, QB))
            return 0
        lax.fori_loop(0, jnp.where((g == NG - UN) & (sb < NSB - 1), 1, 0), next_block, 0)
        return 0
    lax.fori_loop(0, NSB * NG // UN, step, 0)

    acc, seen = ac[...], [chk[0], chk[1], chk[2]]
    for n, c in enumerate((NM - 1, NC - 1)):
        acc = acc + _dot(values_a(c), _bf16(jnp.concatenate([pc[n * NT + j] for j in range(NT)], axis=1)))
    normalize(acc, range(NT), (NSB - 1) % 2, 0, NG - 1, U - 1, seen)
    for j in range(NT):
        output_tile(NT + j, (NSB - 1) % 2, j)
        if j == NT - 2:
            out_copy(NC - NT, NT, NT - 1).start()
    out_copy(NC - 1, 2 * NT - 1, 1).start()

    safe = ((seen[0] >= L_LO) & (seen[1] <= L_HI) | (row8 != 2)) & (jnp.abs(seen[2]) < jnp.inf)
    unsafe = jnp.max(jnp.where(safe, 0, 1))
    for g in range(0, NG, UN):
        out_copy(NC - 2 * NT + g, g, UN).wait()
    out_copy(NC - NT, NT, NT - 1).wait()
    out_copy(NC - 1, 2 * NT - 1, 1).wait()

    def redo(t, _):
        attend_safely(t)
        output_tile(0, 0, 0)
        out_copy(t, 0, 1).start()
        out_copy(t, 0, 1).wait()
        return 0
    lax.fori_loop(0, jnp.where(unsafe > 0, NC, 0), redo, 0)


@jax.jit
def pallas_concat_heads__grouped_kv_mqa__sliding_block__prompt_kernel(
    A_x: jax.Array,
    A_wq: jax.Array,
    A_wk: jax.Array,
    A_wv: jax.Array,
    A_wo: jax.Array,
    B_x: jax.Array,
    B_wqkv: jax.Array,
    B_wo: jax.Array,
):
    hbm = pl.BlockSpec(memory_space=pltpu.HBM)
    vm = pltpu.VMEM
    out = pl.pallas_call(
        functools.partial(_kernel, PACING),
        out_shape=jax.ShapeDtypeStruct((S, 2 * D), BF16),
        in_specs=[hbm] * 8,
        out_specs=hbm,
        scratch_shapes=[
            vm((D, S), BF16), vm((D, S), BF16),
            vm((D, D), BF16), vm((DH, D), BF16), vm((DH, D), BF16),
            vm((D, D), BF16), vm((D, D), BF16), vm((D, 3 * D), BF16),
            vm((DK // 2, QB), I32), vm((3 * D // 2, DK), I32), vm((D, DK), I32),
            vm(((NC + 2) * NG, GR + 8, T), F32), vm((S, T), F32),
            vm((KB0 + VOFF[NC] * DH, T), I32), vm((2, 3 * NT, GR + 8, T), F32),
            vm((2 * NG * 2 + 4, GR + 8, T), F32), vm((2 * H * 2 + 1, T // 2, T), I32),
            vm((2, 2, NT, NG + 1, GR + 8, T), F32), vm((2 * QB, 2 * D), BF16),
            vm((2 * NT, T // 2, T), I32), vm((24, QB), F32), vm((4, 8, T), F32),
            pltpu.SMEM((2,), I32), pltpu.SemaphoreType.DMA((16,)), pltpu.SemaphoreType.DMA((2 * NT,)),
        ],
        compiler_params=pltpu.CompilerParams(vmem_limit_bytes=100 << 20),
        name="fused_attn",
    )(A_x[0].T, A_wq, A_wk.T, A_wv.T, A_wo, B_x[0].T, B_wqkv, B_wo)
    return out[None]
```
